```python
import jax
import jax.numpy as jnp

def _softmax(x, axis=-1):
    return jax.nn.softmax(x, axis=axis)
def _gelu(x):
    return jax.nn.gelu(x, approximate=True)
def _silu(x):
    return jax.nn.silu(x)
def _sigmoid(x):
    return jax.nn.sigmoid(x)
def _layernorm(x, axis=-1, eps=1e-5):
    m = jnp.mean(x, axis=axis, keepdims=True)
    v = jnp.var(x, axis=axis, keepdims=True)
    return (x - m) / jnp.sqrt(v + eps)
def _scatter_add(tgt, idx, src, axis=0):
    return tgt.at[idx].add(src)
def _segment_sum(src, seg, n):
    return jax.ops.segment_sum(src, seg, n)
class _Rng:
    def __init__(self, key):
        self._k = key
    def _next(self):
        self._k, sub = jax.random.split(self._k)
        return sub
    def normal(self, shape):
        return jax.random.normal(self._next(), shape, dtype=jnp.bfloat16)
    def randint(self, lo, hi, shape):
        return jax.random.randint(self._next(), shape, lo, hi, dtype=jnp.int32)
    def uniform(self, shape, lo=0.0, hi=1.0):
        return jax.random.uniform(self._next(), shape, jnp.bfloat16, lo, hi)
    def permutation(self, n):
        return jax.random.permutation(self._next(), n)


kernel_name = 'standalone__structured_sparse_n_m__ragged'

def setup_inputs():
    _rng = _Rng(jax.random.key(int.from_bytes(__import__("os").urandom(4), "little")))
    _w = (lambda a: (lambda t: t.astype(jnp.bfloat16) if jnp.issubdtype(t.dtype, jnp.floating) else t)(jnp.asarray(a)))
    B, S, D = 16, 4096, 576
    assert D % 4 == 0, "d_model must be divisible by M=4 for 2:4 sparsity"
    return {
        "x": _w((lambda *s: _rng.normal(s) * 0.05)(B, S, D)),
        "w": _w((lambda *s: _rng.normal(s) * 0.05)(D, D)),
        "b": _w((lambda *s: _rng.normal(s) * 0.05)(D)),
    }

def reference(x, w, b):
    B, S, D = x.shape
    N, M = 2, 4
    G = D // M
    wg = w.reshape(G, M, D)
    mag = jnp.abs(wg)
    order = jnp.argsort(mag, 1)
    thr = jnp.take_along_axis(mag, order[:, M - N:M - N + 1, :], 1)
    mask = (lambda x, dt: x.astype(dt))(mag >= thr, w.dtype)
    wp = (wg * mask).reshape(D, D)
    return jnp.einsum("bsd,df->bsf", x, wp) + b
```

```python
import jax
import jax.numpy as jnp
from jax import lax
import jax.experimental.pallas as pl
import jax.experimental.pallas.tpu as pltpu

UNIT = 64
HALF = 288
STEP = 256
FIRST = 1024
NX = 9

W_TERMS = {
    "t23": ([(-.5, 1, 0), (-.25, 1, 1)], [(1, 0, 2), (1, 0, 3)]),
    "t32": ([(-.5, 1, 1)], [(-1, 0, 3)]),
    "g0": ([(.25, 0, 0), (-.125, 0, 1), (.25, 1, 0), (.375, 1, 1)], [(1 / 3, 0, 8)]),
    "g1": ([(-.5, 0, 2), (-1, 0, 3), (-.5, 1, 2)], [(-1 / 3, 1, 8)]),
    "t21": ([(.25, 0, 0), (-.125, 0, 1), (-.25, 1, 0), (.125, 1, 1)], [(-1, 0, 7)]),
    "t20": ([(-.5, 0, 2), (.5, 1, 2)], [(-1, 1, 6)]),
    "t31": ([(-.25, 0, 0), (.125, 0, 1), (-.25, 1, 0), (.125, 1, 1)], [(-1, 0, 5)]),
    "t30": ([(.5, 0, 2), (.5, 1, 2)], [(1, 1, 4)]),
    "t10": ([(-1, 0, 4), (1, 1, 4)], [(1, 0, 6), (1, 1, 6)]),
    "t01": ([(-.5, 0, 5), (.5, 1, 5)], [(-1, 0, 7), (-1, 1, 7)]),
    "g2": ([(-.5, 0, 5), (-.5, 1, 4)], [(1 / 3, 0, 8), (1 / 3, 1, 8)]),
    "g3": ([(-1, 0, 7), (1, 1, 6)], [(-1 / 3, 0, 8), (1 / 3, 1, 8)]),
    "t12": ([(.5, 0, 1), (-.5, 1, 1)], [(1, 0, 6), (1, 0, 7)]),
    "t13": ([(.5, 0, 0), (.25, 0, 1), (.5, 1, 0), (.25, 1, 1)], [(1, 0, 4), (1, 0, 5)]),
    "t02": ([(-1, 0, 3), (1, 1, 3)], [(1, 1, 6), (1, 1, 7)]),
    "t03": ([(1, 0, 2), (1, 0, 3), (1, 1, 2), (1, 1, 3)], [(.5, 1, 4), (.5, 1, 5)]),
}
PASSES = list(W_TERMS)
SEGMENTS = [(0, 128, 0, 128), (128, 128, 256, 384), (256, 32, 512, 544)]


def _prune_packed(u):
    mate = lax.broadcasted_iota(jnp.int32, u.shape, 0) ^ 1
    lo = pltpu.bitcast((u << 16) & 0x7FFFFFFF, jnp.float32)
    hi = pltpu.bitcast(u & 0x7FFF0000, jnp.float32)
    big, small = jnp.maximum(lo, hi), jnp.minimum(lo, hi)
    nbig = jnp.take_along_axis(big, mate, axis=0, mode="promise_in_bounds")
    nsmall = jnp.take_along_axis(small, mate, axis=0, mode="promise_in_bounds")
    thr = jnp.maximum(jnp.minimum(big, nbig), jnp.maximum(small, nsmall))
    return u & (jnp.where(lo < thr, 0, 0xFFFF) | jnp.where(hi < thr, 0, -65536))


def _prepare_weights(wbuf, bbuf, a_ref, bias_ref):
    u = pltpu.bitcast(wbuf[...], jnp.int32)
    u = jnp.concatenate([_prune_packed(u[i:i + 8]) for i in range(0, u.shape[0], 8)], axis=0)
    wp = pltpu.bitcast(u, jnp.bfloat16).astype(jnp.float32)
    for p0, n, r0, r1 in SEGMENTS:
        halves = (wp[:, r0:r0 + n], wp[:, r1:r1 + n])
        for t, name in enumerate(PASSES):
            parts = []
            for terms in W_TERMS[name]:
                acc = None
                for c, h, k in terms:
                    v = halves[h][UNIT * k:UNIT * (k + 1)]
                    v = v if c == 1 else v * c
                    acc = v if acc is None else acc + v
                parts.append(acc.astype(jnp.bfloat16))
            a_ref[t, pl.ds(p0 // 2, n // 2), :] = pltpu.bitcast(
                jnp.concatenate(parts, axis=0).T, jnp.int32)
    bias = bbuf[...].reshape(1, 2 * HALF).astype(jnp.float32)
    bias = jnp.broadcast_to(bias, (128, 2 * HALF)).T
    for p0, n, r0, r1 in SEGMENTS:
        bias_ref[p0:p0 + n] = bias[r0:r0 + n]
        bias_ref[HALF + p0:HALF + p0 + n] = bias[r1:r1 + n]


def _token_operands(xa, xb):
    raw = [(xa[UNIT * k:UNIT * (k + 1)], xb[UNIT * k:UNIT * (k + 1)]) for k in range(9)]
    x = [(p.astype(jnp.float32), q.astype(jnp.float32)) for p, q in raw]
    cat = lambda p, q: jnp.concatenate([p.astype(jnp.bfloat16), q.astype(jnp.bfloat16)], axis=0)
    d10, d11 = x[1][0] + x[1][0], x[1][1] + x[1][1]
    e0, f0 = x[0][0] - d11, x[0][1] - d10
    p5, p7 = x[5][0] + x[5][1], x[7][0] + x[7][1]
    e2, e3 = x[4][0] - p5, x[6][0] - p7
    return {
        "t23": cat(x[0][0] + x[0][1], raw[2][0]),
        "t32": cat(e0 + f0, x[2][0] - x[3][0]),
        "g0": cat(e0, raw[8][0]),
        "g1": cat(x[2][0] - x[3][1], x[8][0] + x[8][1]),
        "t21": cat(x[0][0] - x[0][1], x[6][0] - x[7][0]),
        "t20": cat(x[2][0] - x[2][1], e3 + x[6][1]),
        "t31": cat(x[0][1] - d11, x[4][0] - x[5][0]),
        "t30": cat(x[2][1] - x[3][1], e2 + x[4][1]),
        "t10": cat(x[4][0] - x[4][1], raw[6][1]),
        "t01": cat(x[5][0] - x[5][1], raw[7][1]),
        "g2": cat(e2 + x[4][0], raw[8][1]),
        "g3": cat(e3, x[8][0] - x[8][1]),
        "t12": cat(e0 - f0, raw[6][0]),
        "t13": cat(x[0][1] + d11, raw[4][0]),
        "t02": cat(x[3][0] - x[3][1], p7),
        "t03": cat(raw[3][1], p5),
    }


def _multiply(xa, xb, a_ref, bias_ref):
    operands = _token_operands(xa, xb)

    def mm(name):
        a = pltpu.bitcast(a_ref[PASSES.index(name)], jnp.bfloat16)
        return jnp.dot(a, operands[name], preferred_element_type=jnp.float32)

    m23, m32, g0, g1 = mm("t23"), mm("t32"), mm("g0"), mm("g1")
    m23 = m23 + g0 + g1
    m32 = m32 + (g0 + g0) - g1
    m21, m20, m31, m30 = mm("t21"), mm("t20"), mm("t31"), mm("t30")
    y20, y21 = m21 + m23, m20 - m21 + m23
    y30, y31 = m31 + m32, m30 - m31
    c00, c01, c10, c11 = y30 + y20, y31 + y21, y30 - y20, y31 - y21
    m10, m01, g2, g3 = mm("t10"), mm("t01"), mm("g2"), mm("g3")
    m10 = m10 + (g2 + g2) + g3
    m01 = m01 - g2 + g3
    m12, m13, m02, m03 = mm("t12"), mm("t13"), mm("t02"), mm("t03")
    m13 = m13 + bias_ref[0:HALF]
    m03 = m03 + bias_ref[HALF:2 * HALF]
    return ((c00 + m12 + m13, c01 + m10 + m13), (c10 + m01 + m02 + m03, c11 - m01 + m03))


def _kernel(x_hbm, w_hbm, b_hbm, o_hbm, xbuf, obuf, wbuf, bbuf, a_ref, bias_ref,
            xsem, fsem, osem):
    NB, _, S = x_hbm.shape
    steps = S // STEP

    def batch_in(b):
        return pltpu.make_async_copy(x_hbm.at[b], xbuf.at[b % NX], xsem.at[b % NX])

    def first_in(j):
        cols = pl.ds(pl.multiple_of(j * FIRST, FIRST), FIRST)
        return pltpu.make_async_copy(x_hbm.at[0, :, cols], xbuf.at[0, :, cols], fsem.at[2 + j])

    def step_out(b, s):
        return pltpu.make_async_copy(
            obuf.at[b * steps + s], o_hbm.at[b, :, pl.ds(s * STEP, STEP)], osem)

    w_in = pltpu.make_async_copy(w_hbm, wbuf, fsem.at[0])
    b_in = pltpu.make_async_copy(b_hbm, bbuf, fsem.at[1])
    w_in.start()
    b_in.start()
    for j in range(S // FIRST):
        first_in(j).start()
    batch_in(1).start()
    w_in.wait()
    b_in.wait()
    _prepare_weights(wbuf, bbuf, a_ref, bias_ref)
    for b in range(2, NX):
        batch_in(b).start()

    def step(slot, col, dst):
        cols = [pl.ds(pl.multiple_of(col + 128 * j, 128), 128) for j in range(2)]
        out = _multiply(xbuf[slot, :, cols[0]], xbuf[slot, :, cols[1]], a_ref, bias_ref)
        for h in range(2):
            for j in range(2):
                v = out[h][j].astype(obuf.dtype)
                for p0, n, r0, r1 in SEGMENTS:
                    obuf[dst, pl.ds((r0, r1)[h], n), pl.ds(128 * j, 128)] = v[p0:p0 + n]

    def first_batch(j, carry):
        first_in(j).wait()
        for s in range(FIRST // STEP):
            step(0, j * FIRST + s * STEP, j * (FIRST // STEP) + s)
        return carry

    lax.fori_loop(0, S // FIRST, first_batch, 0)
    batch_in(NX).start()

    def batch(b, carry):
        batch_in(b).wait()
        for s in range(steps):
            step(b % NX, s * STEP, b * steps + s)

            @pl.when(b >= NB // 2)
            def _():
                for q in (2 * s, 2 * s + 1):
                    step_out(2 * b - NB + q // steps, q % steps).start()

        @pl.when(b + NX < NB)
        def _():
            batch_in(b + NX).start()
        return carry

    lax.fori_loop(1, NB, batch, 0)
    pltpu.make_async_copy(obuf, obuf, osem).wait()


@jax.jit
def pallas_standalone__structured_sparse_n_m__ragged_kernel(
    x: jax.Array,
    w: jax.Array,
    b: jax.Array,
):
    B, S, D = x.shape
    assert w.shape == (D, D) and D == 9 * UNIT == 2 * HALF
    out = pl.pallas_call(
        _kernel,
        in_specs=[pl.BlockSpec(memory_space=pl.ANY)] * 3,
        out_specs=pl.BlockSpec(memory_space=pl.ANY),
        out_shape=jax.ShapeDtypeStruct((B, D, S), x.dtype),
        scratch_shapes=[
            pltpu.VMEM((NX, D, S), x.dtype),
            pltpu.VMEM((B * S // STEP, D, STEP), x.dtype),
            pltpu.VMEM((D, D), w.dtype),
            pltpu.VMEM((D,), b.dtype),
            pltpu.VMEM((len(PASSES), HALF // 2, 128), jnp.int32),
            pltpu.VMEM((D, 128), jnp.float32),
            pltpu.SemaphoreType.DMA((NX,)),
            pltpu.SemaphoreType.DMA((2 + S // FIRST,)),
            pltpu.SemaphoreType.DMA,
        ],
        compiler_params=pltpu.CompilerParams(
            vmem_limit_bytes=126 * 1024 * 1024,
            disable_bounds_checks=True,
        ),
    )(jnp.transpose(x, (0, 2, 1)), w, b)
    return jnp.transpose(out, (0, 2, 1))
```

```python
import jax
import jax.numpy as jnp
from jax import lax
import jax.experimental.pallas as pl
import jax.experimental.pallas.tpu as pltpu

UNIT = 64
HALF = 288
QUART = 144
STEP = 256
FIRST = 1024
RING = 5
PIECES = 64
READ_AHEAD = 24
EARLY_ROWS = 4
EARLY_STEPS = (1, 4, 7, 10, 13)

PASSES = {
    "cA": ([(.5, 0, 0), (.5, 1, 0)], [(1, 0, 4), (1, 1, 4)]),
    "cB": ([(.25, 0, 0), (-.5, 0, 1)], [(-1, 0, 5)]),
    "dA": ([(.5, 0, 2), (.5, 1, 2)], [(.5, 0, 6), (.5, 1, 6)]),
    "dB": ([(-.5, 0, 3)], [(-1, 0, 7)]),
    "g": ([(-.25, 0, 0), (-.5, 0, 1), (-.5, 1, 0)], [(-1, 0, 2), (-1, 0, 3), (-1, 1, 2)]),
    "h": ([(-.5, 0, 4), (-.5, 0, 5), (-.5, 1, 4)], [(-.5, 0, 6), (-1, 0, 7), (-.5, 1, 6)]),
    "bD": ([(1, 0, 2), (.5, 0, 3)], [(1 / 3, 0, 8)]),
    "bC": ([(.25, 0, 0), (.5, 0, 1)], [(1, 0, 6), (1, 0, 7)]),
    "aC": ([(.5, 0, 0), (1, 0, 1), (.5, 1, 0), (1, 1, 1)],
           [(1, 0, 6), (1, 0, 7), (1, 1, 6), (1, 1, 7)]),
    "aD": ([(1, 0, 2), (.5, 0, 3), (1, 1, 2), (.5, 1, 3)], [(1 / 3, 0, 8), (1 / 3, 1, 8)]),
    "aZ": ([(1, 0, 4), (1, 0, 5), (1, 1, 4), (1, 1, 5)], [(1 / 3, 0, 8), (1 / 3, 1, 8)]),
    "bZ": ([(.5, 0, 4), (.5, 0, 5)], [(1 / 3, 0, 8)]),
}
DEEP = {
    "aB": (([(-.5, 1, 0), (1, 1, 1)], [(-.5, 0, 3), (.5, 1, 3)]),
           ([(-1, 0, 7), (1, 1, 7)], [(-1, 1, 5)])),
    "bA": (([(.5, 1, 0)], [(-.5, 1, 4)]),
           ([(-.5, 0, 2), (.5, 1, 2)], [(-.5, 0, 6), (.5, 1, 6)])),
}
SEGMENTS = [(0, 128, 0, 128), (128, 128, 256, 384), (256, 32, 512, 544)]


def _prune_packed(u):
    mate = lax.broadcasted_iota(jnp.int32, u.shape, 0) ^ 1
    lo = pltpu.bitcast((u << 16) & 0x7FFFFFFF, jnp.float32)
    hi = pltpu.bitcast(u & 0x7FFF0000, jnp.float32)
    big, small = jnp.maximum(lo, hi), jnp.minimum(lo, hi)
    nbig = jnp.take_along_axis(big, mate, axis=0, mode="promise_in_bounds")
    nsmall = jnp.take_along_axis(small, mate, axis=0, mode="promise_in_bounds")
    thr = jnp.maximum(jnp.minimum(big, nbig), jnp.maximum(small, nsmall))
    return u & (jnp.where(lo < thr, 0, 0xFFFF) | jnp.where(hi < thr, 0, -65536))


def _prepare_weights(wbuf, bbuf, long_ref, short_ref, bias_ref):
    u = pltpu.bitcast(wbuf[...], jnp.int32)
    u = jnp.concatenate([_prune_packed(u[i:i + 8]) for i in range(0, u.shape[0], 8)], axis=0)
    wp = pltpu.bitcast(u, jnp.bfloat16).astype(jnp.float32)

    def combine(products, r0, r1, n):
        halves = (wp[:, r0:r0 + n], wp[:, r1:r1 + n])
        parts = []
        for terms in products:
            acc = None
            for c, h, k in terms:
                v = halves[h][UNIT * k:UNIT * (k + 1)]
                v = v if c == 1 else v * c
                acc = v if acc is None else acc + v
            parts.append(acc)
        return jnp.concatenate(parts, axis=0)

    for p0, n, r0, r1 in SEGMENTS:
        for t, products in enumerate(PASSES.values()):
            long_ref[t, pl.ds(p0 // 2, n // 2), :] = pltpu.bitcast(
                combine(products, r0, r1, n).astype(jnp.bfloat16).T, jnp.int32)
    for i, halves in enumerate(DEEP.values()):
        k1, k2 = [jnp.concatenate([combine(products, r0, r1, n).T for _, n, r0, r1 in SEGMENTS],
                                  axis=0) for products in halves]
        a11, a12, a21, a22 = k1[:QUART], k2[:QUART], k1[QUART:], k2[QUART:]
        for t, v in enumerate((a11 + a22, a21 + a22, a11, a21 - a11, a22, a11 + a12, a12 - a22)):
            short_ref[7 * i + t] = pltpu.bitcast(v.astype(jnp.bfloat16), jnp.int32)
    bias = bbuf[...].reshape(1, 2 * HALF).astype(jnp.float32)
    bias = jnp.broadcast_to(bias, (128, 2 * HALF)).T
    for p0, n, r0, r1 in SEGMENTS:
        bias_ref[p0:p0 + n] = bias[r0:r0 + n]
        bias_ref[HALF + p0:HALF + p0 + n] = bias[r1:r1 + n]


def _token_operands(tokens):
    tokens = tokens.astype(jnp.float32)
    x = [(tokens[UNIT * k:UNIT * (k + 1), :128], tokens[UNIT * k:UNIT * (k + 1), 128:])
         for k in range(9)]
    cat = lambda p, q: jnp.concatenate([p, q], axis=0)
    y, z = x[0][0] + x[0][0], x[0][1] + x[0][1]
    cA0, bA0 = y - x[1][0], z + x[1][1]
    bD1 = x[2][0] + x[2][1]
    g1 = bD1 - x[3][0]
    aB1 = x[3][0] + x[3][1] + x[3][1]
    bZ2 = x[4][0] + x[4][1]
    e2 = bZ2 - x[5][0]
    bC3 = x[6][0] + x[6][1]
    h3 = bC3 - x[7][0]
    m8, p8 = x[8][0] - x[8][1], x[8][0] + x[8][1] + x[8][1]
    return {
        "cA": cat(cA0, x[4][0] - x[5][0]),
        "cB": cat(cA0 + (z - x[1][1]), e2 - x[5][1]),
        "dA": cat(x[2][0] - x[3][0] - x[3][0], x[6][0] - x[7][0]),
        "dB": cat(g1 - aB1, h3 - x[7][1]),
        "g": cat(cA0 + bA0, g1),
        "h": cat(e2 - x[5][0], h3),
        "bD": cat(bD1, m8),
        "bC": cat(y + x[1][0] + bA0, bC3),
        "aC": cat(x[1][0], x[7][0]),
        "aD": cat(x[3][0], m8),
        "aZ": cat(x[5][0], p8),
        "bZ": cat(bZ2, p8),
        "aB": (cat(x[1][1], aB1), cat(x[7][1], x[5][0] - x[5][1])),
        "bA": (cat(bA0, x[4][0] - x[4][1]), cat(bD1 + x[2][1], x[6][1])),
    }


def _two_steps(load, store, long_ref, short_ref, bias_ref, midway=None):
    def dot(a, b):
        return jnp.dot(pltpu.bitcast(a, jnp.bfloat16), b.astype(jnp.bfloat16),
                       preferred_element_type=jnp.float32)

    def passes(i, group):
        operands = _token_operands(load(i, group))
        names = list(PASSES)
        return [dot(long_ref[t], operands[names[t]]) for t in range(4 * group, 4 * group + 4)]

    deep = {}
    for j, name in enumerate(DEEP):
        (b11, b21), (b12, b22) = [_token_operands(load(i, 3 + j))[name] for i in range(2)]
        m1, m2, m3, m6 = [dot(short_ref[7 * j + t], v)
                          for t, v in enumerate((b11 + b22, b11, b12 - b22, b11 + b12))]
        c22 = m1 - m2 + m3 + m6
        m4, m5, m7 = [dot(short_ref[7 * j + 4 + t], v)
                      for t, v in enumerate((b21 - b11, b22, b21 + b22))]
        c11, c12, c21 = m1 + m4 - m5 + m7, m3 + m5, m2 + m4
        deep[name] = (jnp.concatenate([c11, c21], axis=0), jnp.concatenate([c12, c22], axis=0))

    for i in range(2):
        cA, cB, dA, dB = passes(i, 0)
        b0, b1 = bias_ref[0:HALF], bias_ref[HALF:2 * HALF]
        s = cA + dA
        c00, c01, c10, c11 = s + b0, cB + dB - s + b0, dA + b1, dB - dA + b1
        g, h, bD, bC = passes(i, 1)
        s = g + h
        aB = deep["aB"][i] - s - h
        u = deep["bA"][i] + s + bD
        v = u + bD + bC
        c00, c01, c10, c11 = c00 + v, c01 - u, c10 - v, c11 + u + aB
        if i == 0 and midway:
            midway()
        aC, aD, aZ, bZ = passes(i, 2)
        s = aZ - bZ
        out = ((c00 + bZ, c01 + bZ), (c10 + aC + aD + aD + s, c11 - aD + s))
        out = [jnp.concatenate(half, axis=1).astype(jnp.bfloat16) for half in out]
        store(i, [((r0, r1)[j], out[j][p0:p0 + n]) for j in range(2) for p0, n, r0, r1 in SEGMENTS])


def _start_when(t, lo, hi, copies):
    for k in range(0, len(copies), 4):
        @pl.when(jnp.logical_and(t >= lo, t + k <= hi + k))
        def _():
            for copy in copies[k:k + 4]:
                copy().start()


def _kernel(x_hbm, w_hbm, b_hbm, o_hbm, xbuf, obuf, wbuf, bbuf, long_ref, short_ref, bias_ref,
            xsem, fsem, osem):
    NB, D, S = x_hbm.shape
    pairs, steps = NB // 2, S // STEP

    def blocks(ref, rows):
        return ref.reshape(ref.shape[0] * D // rows, rows, S)

    def piece(ref, p, j):
        return blocks(ref, 128).at[pl.ds(9 * p, 9), pl.ds(8 * (j // 4), 8),
                                   pl.ds(1024 * (j % 4), 1024)]

    def pair_in(p, slot, j):
        return lambda: pltpu.make_async_copy(
            piece(x_hbm, p, j), piece(xbuf, slot, j), xsem.at[slot])

    def pair_out(p, slot, j):
        return lambda: pltpu.make_async_copy(
            piece(obuf, slot, j), piece(o_hbm, p, j), osem.at[slot])

    def wait_pair(ref, sem, slot):
        view = ref.at[pl.ds(2 * slot, 2)]
        pltpu.make_async_copy(view, view, sem.at[slot]).wait()

    def early_out(i):
        idx = (i // EARLY_ROWS, pl.ds(pl.multiple_of(8 * (i % EARLY_ROWS), 8), 8))
        return pltpu.make_async_copy(
            blocks(obuf, 128).at[idx], blocks(o_hbm, 128).at[idx], osem.at[0])

    def late_out(b, r, c):
        view = lambda ref, i: blocks(ref, 96).at[
            pl.ds(6 * i, 6), pl.ds(8 * r, 8), pl.ds(1024 * c, 1024)]
        return lambda: pltpu.make_async_copy(
            view(obuf, b % (2 * RING)), view(o_hbm, b), osem.at[(b // 2) % RING])

    def last_out(s):
        b, cols = NB - 1, pl.ds(STEP * s, STEP)
        return lambda: pltpu.make_async_copy(
            obuf.at[b % (2 * RING), :, cols], o_hbm.at[b, :, cols], osem.at[(b // 2) % RING])

    def first_in(j):
        cols = pl.ds(pl.multiple_of(j * FIRST, FIRST), FIRST)
        return pltpu.make_async_copy(x_hbm.at[0, :, cols], xbuf.at[0, :, cols], fsem.at[2 + j])

    w_in = pltpu.make_async_copy(w_hbm, wbuf, fsem.at[0])
    b_in = pltpu.make_async_copy(b_hbm, bbuf, fsem.at[1])
    second_in = pltpu.make_async_copy(x_hbm.at[1], xbuf.at[1], xsem.at[0])
    w_in.start()
    b_in.start()
    for j in range(S // FIRST):
        first_in(j).start()
    second_in.start()
    for j in range(READ_AHEAD):
        pair_in(1, 1, j)().start()
    w_in.wait()
    b_in.wait()
    _prepare_weights(wbuf, bbuf, long_ref, short_ref, bias_ref)

    def two_steps(slot, views, col, midway=None, done=None):
        cols = [pl.ds(pl.multiple_of(col + STEP * i, STEP), STEP) for i in range(2)]

        def store(i, parts):
            for r, v in parts:
                obuf[slot, pl.ds(r, v.shape[0]), cols[i]] = v
            if done:
                done(i)

        _two_steps(lambda i, g: xbuf[views[g], :, cols[i]], store,
                   long_ref, short_ref, bias_ref, midway)

    def first_batch(j, carry):
        first_in(j).wait()
        views = [j >> (8 + g) for g in range(5)]
        for col in range(0, FIRST, 2 * STEP):
            two_steps(0, views, j * FIRST + col)
        return carry

    lax.fori_loop(0, S // FIRST, first_batch, 0)

    def batch(t, carry):
        ring = lambda p: jnp.where(p >= RING, p - RING, p)
        slot = jnp.where(t >= 2 * RING, t - 2 * RING, t)
        views = [slot + (t >> (8 + g)) for g in range(5)]

        @pl.when(t == 1)
        def _():
            second_in.wait()

        @pl.when((t & 1) == 0)
        def _():
            wait_pair(xbuf, xsem, slot >> 1)

        @pl.when(jnp.logical_and((t & 1) == 0, t >= 2 * RING))
        def _():
            wait_pair(obuf, osem, slot >> 1)

        def reads(first):
            for d in range(2):
                js = [q % PIECES for q in range(first, first + 8) if q // PIECES == d]
                _start_when(t, 0, pairs - 1 - d, [pair_in(t + d, ring(t + d), j) for j in js])

        def writes(s):
            p, skip = t - pairs, 4 * EARLY_ROWS
            if s == -1:
                q = pairs - 2
                _start_when(p, q, q, [pair_out(q, q % RING, j) for j in range(skip)])
            if s % 2:
                js = range(skip + 4 * (s + 1), skip + 4 * (s + 3))
                _start_when(p, 0, pairs - 2, [pair_out(p, ring(p), j) for j in js if j < PIECES])
                _start_when(p, 0, pairs - 4, [pair_out(p + 1, ring(p + 1), j - PIECES)
                                              for j in js if PIECES <= j < PIECES + skip])
            last = []
            if s < 3:
                last = [late_out(NB - 2, j // 4, j % 4) for j in range(12 * (s + 1), 12 * (s + 2))]
            elif s >= steps - 4:
                last = [last_out(s)]
            elif s % 4 == 3:
                last = [late_out(NB - 1, r, s // 4) for r in range(12)]
            _start_when(t, NB - 1, NB - 1, last)
            if s in EARLY_STEPS:
                i = (t - 1) * len(EARLY_STEPS) + EARLY_STEPS.index(s)

                @pl.when(i < 9 * EARLY_ROWS)
                def _():
                    early_out(i).start()

        writes(-1)
        for s in range(0, steps, 2):
            two_steps(slot, views, STEP * s, lambda: reads(READ_AHEAD + 4 * s),
                      lambda i: writes(s + i))
        return carry

    lax.fori_loop(1, NB, batch, 0)
    for p in range(pairs - RING, pairs):
        wait_pair(obuf, osem, p % RING)


@jax.jit
def pallas_standalone__structured_sparse_n_m__ragged_kernel(
    x: jax.Array,
    w: jax.Array,
    b: jax.Array,
):
    B, S, D = x.shape
    assert (B, S, D) == (16, 4096, 576) and w.shape == (D, D)
    out = pl.pallas_call(
        _kernel,
        in_specs=[pl.BlockSpec(memory_space=pl.ANY)] * 3,
        out_specs=pl.BlockSpec(memory_space=pl.ANY),
        out_shape=jax.ShapeDtypeStruct((B, D, S), x.dtype),
        scratch_shapes=[
            pltpu.VMEM((2 * RING, D, S), x.dtype),
            pltpu.VMEM((2 * RING, D, S), x.dtype),
            pltpu.VMEM((D, D), w.dtype),
            pltpu.VMEM((D,), b.dtype),
            pltpu.VMEM((len(PASSES), HALF // 2, 128), jnp.int32),
            pltpu.VMEM((7 * len(DEEP), QUART // 2, 128), jnp.int32),
            pltpu.VMEM((D, 128), jnp.float32),
            pltpu.SemaphoreType.DMA((RING,)),
            pltpu.SemaphoreType.DMA((2 + S // FIRST,)),
            pltpu.SemaphoreType.DMA((RING,)),
        ],
        compiler_params=pltpu.CompilerParams(
            vmem_limit_bytes=120 * 1024 * 1024,
            disable_bounds_checks=True,
        ),
    )(jnp.transpose(x, (0, 2, 1)), w, b)
    return jnp.transpose(out, (0, 2, 1))
```

```python
import jax
import jax.numpy as jnp
from jax import lax
import jax.experimental.pallas as pl
import jax.experimental.pallas.tpu as pltpu

UNIT = 64
HALF = 288
QUART = 144
STEP = 256
W_PIECES = ((512, 64), (0, 256), (256, 256))
FIRST = (0, 512, 1024, 2048, 4096)
RING = 5
PIECES = 64
SPLIT = 7
QUEUE = 32
READ_LEAD = 6
WRITE_LEAD = 5
PASSES = ("cA", "cB", "dA", "dB", "g", "h", "bD", "bC", "aC", "aD", "aZ", "bZ")
DEEP = ("aB", "bA")


def _prune_packed(u):
    mate = lax.broadcasted_iota(jnp.int32, u.shape, 0) ^ 1
    lo = pltpu.bitcast((u << 16) & 0x7FFFFFFF, jnp.float32)
    hi = pltpu.bitcast(u & 0x7FFF0000, jnp.float32)
    big, small = jnp.maximum(lo, hi), jnp.minimum(lo, hi)
    nbig = jnp.take_along_axis(big, mate, axis=0, mode="promise_in_bounds")
    nsmall = jnp.take_along_axis(small, mate, axis=0, mode="promise_in_bounds")
    thr = jnp.maximum(jnp.minimum(big, nbig), jnp.maximum(small, nsmall))
    return u & (jnp.where(lo < thr, 0, 0xFFFF) | jnp.where(hi < thr, 0, -65536))


def _prepare_weights(wait, wbuf, bbuf, long_ref, short_ref, bias_ref):
    def units(i):
        r0, n = W_PIECES[i]
        wait(i)
        u = pltpu.bitcast(wbuf[r0:r0 + n], jnp.int32)
        u = jnp.concatenate([_prune_packed(u[k:k + 8]) for k in range(0, n // 2, 8)], axis=0)
        return [u[k:k + UNIT // 2] for k in range(0, n // 2, UNIT // 2)]

    def halves(low, high):
        t = pltpu.bitcast(jnp.concatenate([low, high], axis=0), jnp.bfloat16).T
        t = t.astype(jnp.float32)
        return t[:HALF], t[HALF:]

    (u8,) = units(0)
    a08, a18 = halves(u8, u8)
    b8, a8 = a08 * (1 / 3), (a08 + a18) * (1 / 3)
    bias = bbuf[...].reshape(1, 2 * HALF).astype(jnp.float32)
    bias_ref[...] = jnp.broadcast_to(bias, (128, 2 * HALF)).T

    u0, u1, u2, u3 = units(1)
    (a00, a10), (a01, a11) = (a02, a12), (a03, a13) = halves(u0, u2), halves(u1, u3)
    p, q = a00 * .5, a10 * .5
    s = p + a01
    bC0 = s * .5
    cA0, aB0, bA0, cB0, g0, aC0 = p + q, a11 - q, q, bC0 - a01, bC0 + q, s + q + a11
    p, q = a03 * .5, a13 * .5
    s = a02 + a12
    dA1 = s * .5
    dB1, aB1, bD1, g1, aD1, bA1 = p, q - p, a02 + p, s + a03, s + p + q, dA1 - a02

    u4, u5, u6, u7 = units(2)
    (a06, a16), (a07, a17) = (_, a14), (a05, a15) = halves(u6, u4), halves(u7, u5)
    p = a06 + a16
    q = p + a07
    bC3 = a06 + a07
    cA2, cB2, h2, aZ2, bZ2, aB2, bA2 = p, a05, q * .5, q + a15, bC3 * .5, a15, a14 * .5
    dA3 = p * .5
    dB3, h3, aC3, aB3, bA3 = a07, dA3 + a07, aZ2, a17 - a07, (dA3 - a06) * .5

    is_low = lax.broadcasted_iota(jnp.int32, (HALF, 128), 1) < UNIT
    cat = lambda low, high: jnp.where(is_low, low, high)
    up = lambda v: pltpu.roll(v, UNIT, 1)
    weights = {
        "cA": cat(cA0, cA2), "cB": cat(cB0, cB2), "dA": cat(dA3, dA1), "dB": cat(dB3, dB1),
        "g": cat(g0, g1), "h": cat(h3, h2), "bD": cat(b8, bD1), "bC": cat(bC0, up(bC3)),
        "aC": cat(aC0, up(aC3)), "aD": cat(a8, aD1), "aZ": cat(a8, aZ2), "bZ": cat(b8, bZ2),
        "aB": (cat(aB0, aB1), cat(aB3, aB2)), "bA": (cat(bA0, bA2), cat(bA3, bA1)),
    }
    for t, name in enumerate(PASSES):
        long_ref[t] = weights[name].astype(jnp.bfloat16)
    for i, name in enumerate(DEEP):
        k1, k2 = weights[name]
        w11, w12, w21, w22 = k1[:QUART], k2[:QUART], k1[QUART:], k2[QUART:]
        for t, v in enumerate((w11 + w22, w21 + w22, w11, w21 - w11, w22, w11 + w12, w12 - w22)):
            short_ref[7 * i + t] = v.astype(jnp.bfloat16)


def _token_operands(tokens):
    tokens = tokens.astype(jnp.float32)
    x = [(tokens[UNIT * k:UNIT * (k + 1), :128], tokens[UNIT * k:UNIT * (k + 1), 128:])
         for k in range(9)]
    cat = lambda low, high: jnp.concatenate([low, high], axis=0)
    y, z = x[0][0] + x[0][0], x[0][1] + x[0][1]
    cA0, bA0 = y - x[1][0], z + x[1][1]
    bD1 = x[2][0] + x[2][1]
    g1 = bD1 - x[3][0]
    aB1 = x[3][0] + x[3][1] + x[3][1]
    bZ2 = x[4][0] + x[4][1]
    e2 = bZ2 - x[5][0]
    bC3 = x[6][0] + x[6][1]
    h3 = bC3 - x[7][0]
    m8, p8 = x[8][0] - x[8][1], x[8][0] + x[8][1] + x[8][1]
    return {
        "cA": cat(cA0, x[4][0] - x[5][0]),
        "cB": cat(cA0 + (z - x[1][1]), x[5][1] - e2),
        "dA": cat(x[6][0] - x[7][0], x[2][0] - x[3][0] - x[3][0]),
        "dB": cat(x[7][1] - h3, aB1 - g1),
        "g": cat(cA0 + bA0, g1),
        "h": cat(h3, e2 - x[5][0]),
        "bD": cat(m8, bD1),
        "bC": cat(y + x[1][0] + bA0, bC3),
        "aC": cat(x[1][0], x[7][0]),
        "aD": cat(m8, x[3][0]),
        "aZ": cat(p8, x[5][0]),
        "bZ": cat(p8, bZ2),
        "aB": (cat(x[1][1], aB1), cat(x[7][1], x[5][1] - x[5][0])),
        "bA": (cat(bA0, x[4][1] - x[4][0]), cat(x[6][1] + x[6][1], bD1 + x[2][1])),
    }


def _two_steps(load, midway, store, long_ref, short_ref, bias_ref):
    long_ref, short_ref = long_ref.bitcast(jnp.int32), short_ref.bitcast(jnp.int32)

    def dot(a, b):
        return jnp.dot(pltpu.bitcast(a, jnp.bfloat16), b.astype(jnp.bfloat16),
                       preferred_element_type=jnp.float32)

    def passes(i, group):
        operands = _token_operands(load(i, group))
        return [dot(long_ref[t], operands[PASSES[t]]) for t in range(4 * group, 4 * group + 4)]

    deep = {}
    for j, name in enumerate(DEEP):
        (b11, b21), (b12, b22) = [_token_operands(load(i, 3 + j))[name] for i in range(2)]
        m1, m2, m3, m6 = [dot(short_ref[7 * j + t], v)
                          for t, v in enumerate((b11 + b22, b11, b12 - b22, b11 + b12))]
        c22 = m1 - m2 + m3 + m6
        m4, m5, m7 = [dot(short_ref[7 * j + 4 + t], v)
                      for t, v in enumerate((b21 - b11, b22, b21 + b22))]
        c11, c12, c21 = m1 + m4 - m5 + m7, m3 + m5, m2 + m4
        deep[name] = (jnp.concatenate([c11, c21], axis=0), jnp.concatenate([c12, c22], axis=0))

    for i in range(2):
        cA, cB, dA, dB = passes(i, 0)
        b0, b1 = bias_ref[0:HALF], bias_ref[HALF:2 * HALF]
        s = cA + dA
        c00, c01, c10, c11 = s + b0, cB + dB - s + b0, dA + b1, dB - dA + b1
        g, h, bD, bC = passes(i, 1)
        s = g + h
        aB = deep["aB"][i] + s + h
        u = deep["bA"][i] - s + bD
        v = u + bD + bC
        c00, c01, c10, c11 = c00 + v, c01 - u, c10 - v, c11 + u + aB
        midway(i)
        aC, aD, aZ, bZ = passes(i, 2)
        s = aZ - bZ
        out = ((c00 + bZ, c01 + bZ), (c10 + aC + aD + aD + s, c11 - aD + s))
        store(i, [jnp.concatenate(half, axis=1).astype(jnp.bfloat16) for half in out])


def _start_when(t, lo, hi, copies):
    for k in range(0, len(copies), 4):
        @pl.when(jnp.logical_and(t >= lo, t + k <= hi + k))
        def _():
            for start in copies[k:k + 4]:
                start()


def _kernel(x_hbm, w_hbm, b_hbm, o_hbm, xbuf, obuf, wbuf, bbuf, long_ref, short_ref, bias_ref,
            wsem, fsem, xsem, osem):
    NB, D, S = x_hbm.shape
    pairs, steps = NB // 2, S // STEP

    def blocks(ref, rows):
        return ref.reshape(ref.shape[0] * D // rows, rows, S)

    def piece(ref, pair, block, count, row, col):
        return blocks(ref, 128).at[
            pl.ds(9 * pair + block, count), pl.ds(row, 8), pl.ds(1024 * col, 1024)]

    def pair_in(p, slot, row, col, queue):
        span = ((0, SPLIT), (SPLIT, 9 - SPLIT))[queue]
        return lambda: pltpu.make_async_copy(
            piece(x_hbm, p, *span, row, col), piece(xbuf, slot, *span, row, col),
            xsem.at[slot]).start(priority=queue)

    def pair_out(p, slot, j):
        at = ((0, 4), (4, 5))[j // PIECES] + (8 * (j % PIECES // 4), j % 4)
        return lambda: pltpu.make_async_copy(
            piece(obuf, slot, *at), piece(o_hbm, p, *at), osem.at[slot]).start()

    def wait_all(view, sem):
        pltpu.make_async_copy(view, view, sem).wait()

    w_in = [pltpu.make_async_copy(w_hbm.at[pl.ds(r0, n)], wbuf.at[pl.ds(r0, n)], wsem.at[i])
            for i, (r0, n) in enumerate(W_PIECES)]
    b_in = pltpu.make_async_copy(b_hbm, bbuf, wsem.at[len(W_PIECES)])
    second_in = pltpu.make_async_copy(x_hbm.at[1], xbuf.at[1], xsem.at[0])

    def first_in(j, carry):
        cols = pl.ds(pl.multiple_of(512 * j, 512), 512)
        part = sum((512 * j >= c).astype(jnp.int32) for c in FIRST[1:-1])
        pltpu.make_async_copy(x_hbm.at[0, :, cols], xbuf.at[0, :, cols], fsem.at[part]).start()
        return carry

    def wait_first(part):
        wait_all(xbuf.at[0, :, pl.ds(FIRST[part], FIRST[part + 1] - FIRST[part])], fsem.at[part])

    def fill_queue(r, carry):
        for col in range(4):
            pair_in(1, 1, pl.multiple_of(8 * r, 8), col, 1)()
        return carry

    b_in.start()
    for copy in w_in:
        copy.start()
    lax.fori_loop(0, S // 512, first_in, 0)
    second_in.start()
    lax.fori_loop(0, QUEUE // 4, fill_queue, 0)
    b_in.wait()
    _prepare_weights(lambda i: w_in[i].wait(), wbuf, bbuf, long_ref, short_ref, bias_ref)

    def batch(t, carry):
        ring = lambda p: jnp.where(p >= RING, p - RING, p)
        slot = jnp.where(t >= 2 * RING, t - 2 * RING, t)
        both = pl.ds(2 * (slot >> 1), 2)
        views = [slot + (t >> (8 + g)) for g in range(5)]
        in_slots = [ring(t + d) for d in range(2)]
        out_slots = [ring(t - pairs + d) for d in range(2)]

        @pl.when(t == 0)
        def _():
            wait_first(0)

        @pl.when(t == 1)
        def _():
            second_in.wait()

        @pl.when(jnp.logical_and((t & 1) == 0, t > 0))
        def _():
            wait_all(xbuf.at[both], xsem.at[slot >> 1])

        @pl.when(jnp.logical_and((t & 1) == 0, t >= 2 * RING))
        def _():
            wait_all(obuf.at[both], osem.at[slot >> 1])

        def reads(s):
            if STEP * (s + 1) in FIRST[1:-1]:
                @pl.when(t == 0)
                def _():
                    wait_first(FIRST.index(STEP * (s + 1)))
            for first in range(4 * (READ_LEAD + s), 4 * (READ_LEAD + s + 1)):
                for queue in (1, 0):
                    d, j = divmod(first + queue * QUEUE, PIECES)
                    _start_when(t + queue, 1 - first // PIECES + queue, pairs - 1 - d + queue,
                                [pair_in(t + d, in_slots[d], 8 * (j // 4), j % 4, queue)])

        def writes(s):
            p = t - pairs
            if s < steps - 1:
                d, j = divmod(8 * (WRITE_LEAD + s + 1), 2 * PIECES)
                _start_when(p, -d, pairs - 2 - d,
                            [pair_out(p + d, out_slots[d], j + k) for k in range(8)])
            sem = osem.at[(pairs - 1) % RING]
            if s > 0 and s % 4 == 3:
                view = lambda ref, b, r: blocks(ref, 96).at[
                    pl.ds(6 * b, 6), pl.ds(8 * r, 8), pl.ds(1024 * (s // 4), 1024)]
                _start_when(t, NB - 2, NB - 1 - (s == steps - 1), [
                    lambda r=r: pltpu.make_async_copy(
                        view(obuf, slot, r), view(o_hbm, t, r), sem).start() for r in range(12)])
            if s >= steps - 4:
                cols = pl.ds(STEP * s, STEP)
                _start_when(t, NB - 1, NB - 1, [lambda: pltpu.make_async_copy(
                    obuf.at[slot, :, cols], o_hbm.at[t, :, cols], sem).start()])

        writes(-1)
        for s in range(0, steps, 2):
            def store(i, halves):
                for j, v in enumerate(halves):
                    obuf[slot, pl.ds(HALF * j, HALF), pl.ds(STEP * (s + i), STEP)] = v
                writes(s + i)

            _two_steps(lambda i, g: xbuf[views[g], :, pl.ds(STEP * (s + i), STEP)],
                       lambda i: reads(s + i), store, long_ref, short_ref, bias_ref)
        return carry

    lax.fori_loop(0, NB, batch, 0)
    for p in range(pairs - RING, pairs):
        wait_all(obuf.at[pl.ds(2 * (p % RING), 2)], osem.at[p % RING])


@jax.jit
def pallas_standalone__structured_sparse_n_m__ragged_kernel(
    x: jax.Array,
    w: jax.Array,
    b: jax.Array,
):
    B, S, D = x.shape
    assert (B, S, D) == (16, 4096, 576) and w.shape == (D, D)
    out = pl.pallas_call(
        _kernel,
        in_specs=[pl.BlockSpec(memory_space=pl.ANY)] * 3,
        out_specs=pl.BlockSpec(memory_space=pl.ANY),
        out_shape=jax.ShapeDtypeStruct((B, D, S), x.dtype),
        scratch_shapes=[
            pltpu.VMEM((2 * RING, D, S), x.dtype),
            pltpu.VMEM((2 * RING, D, S), x.dtype),
            pltpu.VMEM((D, D), w.dtype),
            pltpu.VMEM((D,), b.dtype),
            pltpu.VMEM((len(PASSES), HALF, 128), jnp.bfloat16),
            pltpu.VMEM((7 * len(DEEP), QUART, 128), jnp.bfloat16),
            pltpu.VMEM((D, 128), jnp.float32),
            pltpu.SemaphoreType.DMA((len(W_PIECES) + 1,)),
            pltpu.SemaphoreType.DMA((len(FIRST) - 1,)),
            pltpu.SemaphoreType.DMA((RING,)),
            pltpu.SemaphoreType.DMA((RING,)),
        ],
        compiler_params=pltpu.CompilerParams(
            vmem_limit_bytes=120 * 1024 * 1024,
            disable_bounds_checks=True,
            disable_semaphore_checks=True,
            flags={"XLA_TPU_RESCHEDULE_DMA_DONES": True},
        ),
    )(jnp.transpose(x, (0, 2, 1)), w, b)
    return jnp.transpose(out, (0, 2, 1))
```

```python
import jax
import jax.numpy as jnp
from jax import lax
import jax.experimental.pallas as pl
import jax.experimental.pallas.tpu as pltpu

UNIT = 64
HALF = 288
QUART = 144
STEP = 256
W_PIECES = ((512, 64), (0, 256), (256, 256))
FIRST = (0, 512, 1024, 1536, 2048, 3072, 4096)
RING = 5
READ_LEAD = 5
WRITE_LEAD = 5
COVER = 4
PASSES = ("aZ", "bZ", "aC", "aD", "dA", "dB", "cA", "cB", "g", "h", "bD", "bC")
DEEP = ("aB", "bA")


def _prune_packed(u):
    mate = lax.broadcasted_iota(jnp.int32, u.shape, 0) ^ 1
    lo = pltpu.bitcast((u << 16) & 0x7FFFFFFF, jnp.float32)
    hi = pltpu.bitcast(u & 0x7FFF0000, jnp.float32)
    big, small = jnp.maximum(lo, hi), jnp.minimum(lo, hi)
    nbig = jnp.take_along_axis(big, mate, axis=0, mode="promise_in_bounds")
    nsmall = jnp.take_along_axis(small, mate, axis=0, mode="promise_in_bounds")
    thr = jnp.maximum(jnp.minimum(big, nbig), jnp.maximum(small, nsmall))
    return u & (jnp.where(lo < thr, 0, 0xFFFF) | jnp.where(hi < thr, 0, -65536))


def _prepare_weights(wait, wbuf, bbuf, long_ref, short_ref, bias_ref):
    def units(i):
        r0, n = W_PIECES[i]
        wait(i)
        u = pltpu.bitcast(wbuf[r0:r0 + n], jnp.int32)
        u = jnp.concatenate([_prune_packed(u[k:k + 8]) for k in range(0, n // 2, 8)], axis=0)
        return [u[k:k + UNIT // 2] for k in range(0, n // 2, UNIT // 2)]

    def halves(low, high):
        t = pltpu.bitcast(jnp.concatenate([low, high], axis=0), jnp.bfloat16).T
        t = t.astype(jnp.float32)
        return t[:HALF], t[HALF:]

    (u8,) = units(0)
    a08, a18 = halves(u8, u8)
    b8, a8 = a08 * (1 / 3), (a08 + a18) * (1 / 3)
    bias = bbuf[...].reshape(1, 2 * HALF).astype(jnp.float32)
    bias_ref[...] = jnp.broadcast_to(bias, (128, 2 * HALF)).T

    u0, u1, u2, u3 = units(1)
    (a00, a10), (a01, a11) = (a02, a12), (a03, a13) = halves(u0, u2), halves(u1, u3)
    p, q = a00 * .5, a10 * .5
    s = p + a01
    bC0 = s * .5
    cA0, aB0, bA0, cB0, g0, aC0 = p + q, a11 - q, q, bC0 - a01, bC0 + q, s + q + a11
    p, q = a03 * .5, a13 * .5
    s = a02 + a12
    dA1 = s * .5
    dB1, aB1, bD1, g1, aD1, bA1 = p, q - p, a02 + p, s + a03, s + p + q, dA1 - a02

    u4, u5, u6, u7 = units(2)
    (a06, a16), (a07, a17) = (_, a14), (a05, a15) = halves(u6, u4), halves(u7, u5)
    p = a06 + a16
    q = p + a07
    bC3 = a06 + a07
    cA2, cB2, h2, aZ2, bZ2, aB2, bA2 = p, a05, q * .5, q + a15, bC3 * .5, a15, a14 * .5
    dA3 = p * .5
    dB3, h3, aC3, aB3, bA3 = a07, dA3 + a07, aZ2, a17 - a07, (dA3 - a06) * .5

    is_low = lax.broadcasted_iota(jnp.int32, (HALF, 128), 1) < UNIT
    cat = lambda low, high: jnp.where(is_low, low, high)
    up = lambda v: pltpu.roll(v, UNIT, 1)
    weights = {
        "cA": cat(cA0, cA2), "cB": cat(cB0, cB2), "dA": cat(dA3, dA1), "dB": cat(dB3, dB1),
        "g": cat(g0, g1), "h": cat(h3, h2), "bD": cat(b8, bD1), "bC": cat(bC0, up(bC3)),
        "aC": cat(aC0, up(aC3)), "aD": cat(a8, aD1), "aZ": cat(a8, aZ2), "bZ": cat(b8, bZ2),
        "aB": (cat(aB0, aB1), cat(aB3, aB2)), "bA": (cat(bA0, bA2), cat(bA3, bA1)),
    }
    for t, name in enumerate(PASSES):
        long_ref[t] = weights[name].astype(jnp.bfloat16)
    for i, name in enumerate(DEEP):
        k1, k2 = weights[name]
        w11, w12, w21, w22 = k1[:QUART], k2[:QUART], k1[QUART:], k2[QUART:]
        for t, v in enumerate((w11 + w22, w21 + w22, w11, w21 - w11, w22, w11 + w12, w12 - w22)):
            short_ref[7 * i + t] = v.astype(jnp.bfloat16)


def _token_operands(tokens):
    tokens = tokens.astype(jnp.float32)
    x = [(tokens[UNIT * k:UNIT * (k + 1), :128], tokens[UNIT * k:UNIT * (k + 1), 128:])
         for k in range(9)]
    cat = lambda low, high: jnp.concatenate([low, high], axis=0)
    y, z = x[0][0] + x[0][0], x[0][1] + x[0][1]
    cA0, bA0 = y - x[1][0], z + x[1][1]
    bD1 = x[2][0] + x[2][1]
    g1 = bD1 - x[3][0]
    aB1 = x[3][0] + x[3][1] + x[3][1]
    bZ2 = x[4][0] + x[4][1]
    e2 = bZ2 - x[5][0]
    bC3 = x[6][0] + x[6][1]
    h3 = bC3 - x[7][0]
    m8, p8 = x[8][0] - x[8][1], x[8][0] + x[8][1] + x[8][1]
    return {
        "cA": cat(cA0, x[4][0] - x[5][0]),
        "cB": cat(cA0 + (z - x[1][1]), x[5][1] - e2),
        "dA": cat(x[6][0] - x[7][0], x[2][0] - x[3][0] - x[3][0]),
        "dB": cat(x[7][1] - h3, aB1 - g1),
        "g": cat(cA0 + bA0, g1),
        "h": cat(h3, e2 - x[5][0]),
        "bD": cat(m8, bD1),
        "bC": cat(y + x[1][0] + bA0, bC3),
        "aC": cat(x[1][0], x[7][0]),
        "aD": cat(m8, x[3][0]),
        "aZ": cat(p8, x[5][0]),
        "bZ": cat(p8, bZ2),
        "aB": (cat(x[1][1], aB1), cat(x[7][1], x[5][1] - x[5][0])),
        "bA": (cat(bA0, x[4][1] - x[4][0]), cat(x[6][1] + x[6][1], bD1 + x[2][1])),
    }


def _two_steps(load, before, store, long_ref, short_ref, bias_ref):
    long_ref, short_ref = long_ref.bitcast(jnp.int32), short_ref.bitcast(jnp.int32)

    def dot(a, b):
        return jnp.dot(pltpu.bitcast(a, jnp.bfloat16), b.astype(jnp.bfloat16),
                       preferred_element_type=jnp.float32)

    def passes(i, group):
        before(i, group)
        operands = _token_operands(load(i, group))
        return [dot(long_ref[t], operands[PASSES[t]]) for t in range(4 * group, 4 * group + 4)]

    deep = {}
    for j, name in enumerate(DEEP):
        (b11, b21), (b12, b22) = [_token_operands(load(i, 3 + j))[name] for i in range(2)]
        m1, m2, m3, m6 = [dot(short_ref[7 * j + t], v)
                          for t, v in enumerate((b11 + b22, b11, b12 - b22, b11 + b12))]
        c22 = m1 - m2 + m3 + m6
        m4, m5, m7 = [dot(short_ref[7 * j + 4 + t], v)
                      for t, v in enumerate((b21 - b11, b22, b21 + b22))]
        c11, c12, c21 = m1 + m4 - m5 + m7, m3 + m5, m2 + m4
        deep[name] = (jnp.concatenate([c11, c21], axis=0), jnp.concatenate([c12, c22], axis=0))

    for i in range(2):
        aZ, bZ, aC, aD = passes(i, 0)
        b0, b1 = bias_ref[0:HALF], bias_ref[HALF:2 * HALF]
        s = aZ - bZ + b1
        c00 = c01 = bZ + b0
        c10, c11 = aC + aD + aD + s, s - aD
        dA, dB, cA, cB = passes(i, 1)
        s = dB - dA
        c00, c01, c10, c11 = c00 + dA + cA, c01 + s + (cB - cA), c10 + dA, c11 + s
        g, h, bD, bC = passes(i, 2)
        s = g + h
        aB = deep["aB"][i] + s + h
        u = deep["bA"][i] - s + bD
        v = u + (bD + bC)
        out = ((c00 + v, c01 - u), (c10 - v, c11 + aB + u))
        store(i, [jnp.concatenate(half, axis=1).astype(jnp.bfloat16) for half in out])


def _start_when(t, lo, hi, copies):
    for k in range(0, len(copies), 4):
        @pl.when(jnp.logical_and(t >= lo, t + k <= hi + k))
        def _():
            for start in copies[k:k + 4]:
                start()


def _kernel(x_hbm, w_hbm, b_hbm, o_hbm, xbuf, obuf, wbuf, bbuf, long_ref, short_ref, bias_ref,
            wsem, fsem, xsem, osem):
    NB, D, S = x_hbm.shape
    pairs, steps = NB // 2, S // STEP
    out_sem = osem.at[(pairs - 1) % RING]

    def piece(ref, height, block, blocks, row, col, cols, rows=8):
        view = ref.reshape(ref.shape[0] * D // height, height, S)
        return view.at[pl.ds(block, blocks), pl.ds(row, rows), pl.ds(col, cols)]

    def copy_in(height, src, dst, shape, sem, queue):
        return lambda: pltpu.make_async_copy(
            piece(x_hbm, height, src, *shape), piece(xbuf, height, dst, *shape),
            sem).start(priority=queue)

    def copy_out(height, src, dst, shape, sem):
        return lambda: pltpu.make_async_copy(
            piece(obuf, height, src, *shape), piece(o_hbm, height, dst, *shape), sem).start()

    def pair_out(p, slot, r, block=0, blocks=9):
        return [copy_out(128, 9 * slot + block, 9 * p + block, (blocks, 8 * r, col, 1024),
                         osem.at[slot]) for col in range(0, S, 1024)]

    def step_out(s):
        return copy_out(D, (NB - 1) % (2 * RING), NB - 1, (1, 0, STEP * s, STEP, D), out_sem)

    def wait_all(view, sem):
        pltpu.make_async_copy(view, view, sem).wait()

    def wait_first(part):
        wait_all(xbuf.at[0, :, pl.ds(FIRST[part], FIRST[part + 1] - FIRST[part])], fsem.at[part])

    def times(n, i):
        return n * i if isinstance(i, int) else pl.multiple_of(n * i, n)

    def first_quarter(i, carry):
        copy_in(D, 0, 0, (1, 0, times(512, i), 512, D), fsem.at[i], 0)()
        return carry

    def fill_queue(r, carry):
        for col in range(0, S, 1024):
            copy_in(128, 7, 7, (2, times(8, r), col, 1024), xsem.at[0], 1)()
        return carry

    def first_rest(r, k):
        copy_in(128, 5, 5, (2, times(8, r), 1408 * k, min(1408, S - 1408 * k)), xsem.at[0], 1)()
        j = 3 * r + k

        @pl.when(j < 8)
        def _():
            copy_in(64, 0, 0, (9, times(16, j & 3), times(512, 2 + (j >> 2)), 512, 16),
                    fsem.at[2 + (j >> 2)], 0)()

        @pl.when(j >= 8)
        def _():
            copy_in(64, 0, 0, (9, times(8, j & 7), times(1024, 1 + (j >> 3)), 1024),
                    fsem.at[3 + (j >> 3)], 0)()

    def first_rows(r, carry):
        for k in range(3):
            first_rest(r, k)
        return carry

    w_in = [pltpu.make_async_copy(w_hbm.at[pl.ds(r0, n)], wbuf.at[pl.ds(r0, n)], wsem.at[i])
            for i, (r0, n) in enumerate(W_PIECES)]
    b_in = pltpu.make_async_copy(b_hbm, bbuf, wsem.at[len(W_PIECES)])
    b_in.start()
    for copy in w_in:
        copy.start()
    lax.fori_loop(0, 2, first_quarter, 0)
    lax.fori_loop(0, 8, fill_queue, 0)
    lax.fori_loop(0, 7, first_rows, 0)
    b_in.wait()
    _prepare_weights(lambda i: w_in[i].wait(), wbuf, bbuf, long_ref, short_ref, bias_ref)

    def batch(t, slot):
        ring = lambda p: jnp.where(p >= RING, p - RING, p)
        next_slot = jnp.where(t + 1 >= 2 * RING, t + 1 - 2 * RING, t + 1)
        views = [slot + (t >> (8 + g)) for g in range(4)]
        views.insert(3, slot)
        this, then = ring(t), ring(t + 1)
        last = t == pairs - 1
        ahead = jnp.where(last, this, then)
        ahead_src = jnp.where(last, 9 * t + 5, 9 * t + 16)
        ahead_dst = 9 * ahead + jnp.where(last, 5, 7)
        ahead_row = jnp.where(last, 64, 0)
        five = jnp.where(last, 0, 4)
        p = t - pairs
        out_slots = [ring(p), ring(p + 1)]

        @pl.when(t == 0)
        def _():
            wait_first(0)

        @pl.when(jnp.logical_and((t & 1) == 0, t >= 2 * RING))
        def _():
            wait_all(obuf.at[pl.ds(slot, 2)], osem.at[slot >> 1])

        def read(j):
            row, col = 8 * (j % 64 // 4), 1024 * (j % 4)
            if j < 32:
                if j >= 29:
                    pl.when(t + j == j)(lambda: first_rest(7, j - 29))
                _start_when(t + 1, 2, pairs, [copy_in(
                    128, 9 * t + 7, 9 * this + 7, (2, row + 64, col, 1024), xsem.at[this], 1)])
                _start_when(t, 1, pairs - 1, [copy_in(
                    128, 9 * t, 9 * this, (7, row, col, 1024), xsem.at[this], 0)])
            elif j < 64:
                at = pl.multiple_of(ahead_row + row - 64, 8)
                _start_when(t, 0, pairs - 1, [copy_in(
                    128, ahead_src, ahead_dst, (2, at, col, 1024), xsem.at[ahead], 1)])
                _start_when(t, 1, pairs - 2, [copy_in(
                    128, 9 * t, 9 * this, (7, row, col, 1024), xsem.at[this], 0)])
                pl.when(jnp.logical_or(t == 0, last))(copy_in(
                    128, 9 * t + five, 9 * this + five, (5, row, col, 1024), xsem.at[this], 0))
            else:
                _start_when(t + 1, 1, pairs - 1, [copy_in(
                    128, 9 * t + 16, 9 * then + 7, (2, row + 64, col, 1024), xsem.at[then], 1)])
                _start_when(t, 0, pairs - 2, [copy_in(
                    128, 9 * t + 9, 9 * then, (7, row, col, 1024), xsem.at[then], 0)])

        def write(s):
            q = pairs - 2
            r = s + 1 + WRITE_LEAD - steps
            if 0 <= r < COVER:
                _start_when(p, q - 1, q - 1, pair_out(q, q % RING, r, 0, 4))
            if s + 1 < WRITE_LEAD:
                span = (4, 5) if s + 1 < COVER else (0, 9)
                _start_when(p, q, q, pair_out(q, q % RING, s + 1, *span))
            if s + 1 < steps:
                d, r = divmod(s + 1 + WRITE_LEAD, steps)
                _start_when(p, -d, q - 2 * d, pair_out(p + d, out_slots[d], r))
            half = lambda src, dst, h, r: [
                copy_out(64, 9 * src, 9 * dst, (9, 8 * (r + k // 4), 2048 * h + 512 * (k % 4), 512),
                         out_sem) for k in range(8)]
            if s < 3:
                _start_when(t, NB - 1, NB - 1, half((NB - 2) % (2 * RING), NB - 2, 1, 2 * (s + 1)))
            if 7 <= s < 11:
                _start_when(t, NB - 2, NB - 1, half(slot, t, 0, 2 * (s - 7)))
            if s == 11:
                _start_when(t, NB - 1, NB - 1, [
                    copy_out(96, 6 * ((NB - 1) % (2 * RING)), 6 * (NB - 1), (6, row, 2048, 1024),
                             out_sem) for row in range(0, 96, 8)])
            if 12 <= s < steps - 1:
                _start_when(t, NB - 1, NB - 1, [step_out(s)])

        write(-1)
        for s in range(0, steps, 2):
            def before(i, group):
                if (i, group) == (1, 1) and STEP * (s + 2) in FIRST[1:-1]:
                    pl.when(t == 0)(lambda: wait_first(FIRST.index(STEP * (s + 2))))
                if group < 2:
                    for k in range(2):
                        read(4 * (READ_LEAD + s + i) + 2 * group + k)

            def store(i, halves):
                if s + i == steps - 1:
                    pl.when(t == 0)(lambda: wait_all(xbuf.at[1], xsem.at[0]))
                    pl.when(jnp.logical_and((t & 1) == 1, t + 1 < NB))(
                        lambda: wait_all(xbuf.at[pl.ds(next_slot, 2)], xsem.at[next_slot >> 1]))
                for j, v in enumerate(halves):
                    obuf[slot, pl.ds(HALF * j, HALF), pl.ds(STEP * (s + i), STEP)] = v
                write(s + i)

            _two_steps(lambda i, g: xbuf[views[g], :, pl.ds(STEP * (s + i), STEP)],
                       before, store, long_ref, short_ref, bias_ref)
        return next_slot

    lax.fori_loop(0, NB, batch, jnp.int32(0))
    step_out(steps - 1)()
    for p in range(pairs - RING, pairs):
        wait_all(obuf.at[pl.ds(2 * (p % RING), 2)], osem.at[p % RING])


@jax.jit
def pallas_standalone__structured_sparse_n_m__ragged_kernel(
    x: jax.Array,
    w: jax.Array,
    b: jax.Array,
):
    B, S, D = x.shape
    assert (B, S, D) == (16, 4096, 576) and w.shape == (D, D)
    out = pl.pallas_call(
        _kernel,
        in_specs=[pl.BlockSpec(memory_space=pl.ANY)] * 3,
        out_specs=pl.BlockSpec(memory_space=pl.ANY),
        out_shape=jax.ShapeDtypeStruct((B, D, S), x.dtype),
        scratch_shapes=[
            pltpu.VMEM((2 * RING, D, S), x.dtype),
            pltpu.VMEM((2 * RING, D, S), x.dtype),
            pltpu.VMEM((D, D), w.dtype),
            pltpu.VMEM((D,), b.dtype),
            pltpu.VMEM((len(PASSES), HALF, 128), jnp.bfloat16),
            pltpu.VMEM((7 * len(DEEP), QUART, 128), jnp.bfloat16),
            pltpu.VMEM((D, 128), jnp.float32),
            pltpu.SemaphoreType.DMA((len(W_PIECES) + 1,)),
            pltpu.SemaphoreType.DMA((len(FIRST) - 1,)),
            pltpu.SemaphoreType.DMA((RING,)),
            pltpu.SemaphoreType.DMA((RING,)),
        ],
        compiler_params=pltpu.CompilerParams(
            vmem_limit_bytes=120 * 1024 * 1024,
            disable_bounds_checks=True,
            disable_semaphore_checks=True,
            flags={"XLA_TPU_RESCHEDULE_DMA_DONES": True},
        ),
    )(jnp.transpose(x, (0, 2, 1)), w, b)
    return jnp.transpose(out, (0, 2, 1))
```
